```python
import os as _os
_os.environ.setdefault("JAX_PLATFORMS", "cpu")
import jax
import jax.numpy as jnp

def _softmax(x, axis=-1):
    return jax.nn.softmax(x, axis=axis)
def _gelu(x):
    return jax.nn.gelu(x, approximate=True)
def _silu(x):
    return jax.nn.silu(x)
def _sigmoid(x):
    return jax.nn.sigmoid(x)
def _layernorm(x, axis=-1, eps=1e-5):
    m = jnp.mean(x, axis=axis, keepdims=True)
    v = jnp.var(x, axis=axis, keepdims=True)
    return (x - m) / jnp.sqrt(v + eps)
def _scatter_add(tgt, idx, src, axis=0):
    return tgt.at[idx].add(src)
def _segment_sum(src, seg, n):
    return jax.ops.segment_sum(src, seg, n)
class _Rng:
    def __init__(self, key):
        self._k = key
    def _next(self):
        self._k, sub = jax.random.split(self._k)
        return sub
    def normal(self, shape):
        return jax.random.normal(self._next(), shape, dtype=jnp.bfloat16)
    def randint(self, lo, hi, shape):
        return jax.random.randint(self._next(), shape, lo, hi, dtype=jnp.int32)
    def uniform(self, shape, lo=0.0, hi=1.0):
        return jax.random.uniform(self._next(), shape, jnp.bfloat16, lo, hi)
    def permutation(self, n):
        return jax.random.permutation(self._next(), n)


kernel_name = 'parallel_sum__ssm_conv_h3__dense_activation_silu__prompt'

def setup_inputs():
    _rng = _Rng(jax.random.key(int.from_bytes(__import__("os").urandom(4), "little")))
    _w = (lambda a: (lambda t: t.astype(jnp.bfloat16) if jnp.issubdtype(t.dtype, jnp.floating) else t)(jnp.asarray(a)))
    def _A_setup():
        B, S, D = 1, 2048, 448
        ks = 4
        return {
            "q": _w((lambda *s: _rng.normal(s) * 0.05)(B, S, D)),
            "k": _w((lambda *s: _rng.normal(s) * 0.2)(B, S, D)),
            "v": _w((lambda *s: _rng.normal(s) * 0.2)(B, S, D)),
            "shift_k": _w((lambda *s: _rng.normal(s) * 0.2)(D, ks) * 0.5),
            "ssm_k": _w((lambda *s: _rng.normal(s) * 0.2)(D, S) * (1.0 / S ** 0.5)),
            "ssm_D": _w((lambda *s: _rng.normal(s) * 0.2)(D)),
        }
    _A_in = _A_setup()

    def _B_setup():
        B, S, D, F = 1, 2048, 448, 1792
        return {
            "x": _w((lambda *s: _rng.normal(s) * 0.05)(B, S, D)),
            "w1": _w((lambda *s: _rng.normal(s) * 0.05)(D, F) * (D ** -0.5)),
            "w2": _w((lambda *s: _rng.normal(s) * 0.05)(F, D) * (F ** -0.5)),
        }
    _B_in = _B_setup()

    return {
        "A_q": _A_in["q"],
        "A_k": _A_in["k"],
        "A_v": _A_in["v"],
        "A_shift_k": _A_in["shift_k"],
        "A_ssm_k": _A_in["ssm_k"],
        "A_ssm_D": _A_in["ssm_D"],
        "B_x": _B_in["x"],
        "B_w1": _B_in["w1"],
        "B_w2": _B_in["w2"],
    }

def reference(A_q, A_k, A_v, A_shift_k, A_ssm_k, A_ssm_D, B_x, B_w1, B_w2):
    def _A_ref(q, k, v, shift_k, ssm_k, ssm_D):
        B, S, D = q.shape
        ks = shift_k.shape[-1]
        k_pad = jnp.pad(k, ((0, 0), (ks - 1, 0), (0, 0)))
        k_shift = jnp.zeros_like(k)
        for t in range(ks):
            k_shift = k_shift + k_pad[:, t:t + S, :] * shift_k[:, ks - 1 - t][None, None, :]
        kv = k_shift * v
        L = 2 * S
        kv_pad = jnp.pad(kv, ((0, 0), (0, S), (0, 0)))
        kf_pad = jnp.pad(ssm_k, ((0, 0), (0, S)))
        kv_f = (lambda x, axes=(-2,-1): jnp.fft.rfft2(x.astype(jnp.float32), axes=axes))(kv_pad[:, None, :, :], axes=(1, 2))
        kf_f = (lambda x, axes=(-2,-1): jnp.fft.rfft2(x.astype(jnp.float32), axes=axes))(kf_pad[:, None, :], axes=(1, 2))
        kf_f = (lambda x, *d: x.transpose(*d))(kf_f, 1, 2, 0)
        y_f = kv_f * kf_f[None, :, :, :]
        y = (lambda x, s, axes=(-2,-1): jnp.fft.irfft2(x, s=s, axes=axes).astype(jnp.bfloat16))(y_f, (1, L), axes=(1, 2))[:, 0, :S, :]
        y = y + kv * ssm_D[None, None, :]
        return q * y

    def _B_ref(x, w1, w2):
        h = jnp.einsum("bsd,df->bsf", x, w1)
        h = _silu(h)
        out = jnp.einsum("bsf,fd->bsd", h, w2)
        return out

    x = A_q
    xn = _layernorm(x, axis=-1)
    return x + _A_ref(xn, A_k, A_v, A_shift_k, A_ssm_k, A_ssm_D) + _B_ref(xn, B_w1, B_w2)
```

```python
import numpy as np
import jax
import jax.numpy as jnp
from jax import lax
import jax.experimental.pallas as pl
import jax.experimental.pallas.tpu as pltpu
import ml_dtypes

SEQ = 2048; D = 448; FF = 1792
N1 = 128; N2 = 4; NBK = 4; L = 512
NT = 4
TT = 16
KF = 14
EPS = 1e-5
DH = D//2
YP = 0

f32 = jnp.float32; bf16 = jnp.bfloat16; u32 = jnp.uint32

def _env(name, default):
    return {'G4': '6'}.get(name, default)

def _pack_rows(a):
    b = np.ascontiguousarray(a.astype(ml_dtypes.bfloat16)).view(np.uint16).astype(np.uint32)
    return np.ascontiguousarray(b[..., 0::2, :] | (b[..., 1::2, :] << 16))

def _tables():
    n1 = np.arange(N1); k1 = np.arange(N1)
    F = np.zeros((N2, 2*N1, N1), np.float64)
    G = np.zeros((N2, N1, 2*N1), np.float64)
    col_re = (k1//8)*16 + 2*(k1 % 8)
    col_im = col_re + 1
    for n2 in range(N2):
        e = ((N2*n1[None, :] + n2) * (4*k1[:, None] + 1)) % (4*L)
        th = 2*np.pi*e/(4*L)
        c = np.cos(th); s = np.sin(th)
        F[n2, :N1] = c; F[n2, N1:] = s
        G[n2][:, col_re] = c.T / L
        G[n2][:, col_im] = s.T / L
    G = G.reshape(N2, N1, 2, 128).transpose(0, 2, 1, 3)
    return _pack_rows(F).reshape(N2*128, 128), _pack_rows(G).reshape(N2*2*64, 128)

_F, _G = _tables()

def c0_of(ct):
    return min(128*ct, D - 128)

def cadd(a, b): return (a[0] + b[0], a[1] + b[1])
def csub(a, b): return (a[0] - b[0], a[1] - b[1])
def cmul(a, b): return (a[0]*b[0] - a[1]*b[1], a[0]*b[1] + a[1]*b[0])
def dft4(x, s):
    s0 = cadd(x[0], x[2]); s1 = csub(x[0], x[2])
    s2 = cadd(x[1], x[3]); s3 = csub(x[1], x[3])
    if s > 0:
        o1 = (s1[0] - s3[1], s1[1] + s3[0]); o3 = (s1[0] + s3[1], s1[1] - s3[0])
    else:
        o1 = (s1[0] + s3[1], s1[1] - s3[0]); o3 = (s1[0] - s3[1], s1[1] + s3[0])
    return [cadd(s0, s2), o1, csub(s0, s2), o3]

_off = [0]
def _reg(n):
    o = _off[0]; _off[0] += n; return o
R_XN = _reg(TT*256)
R_W1T = _reg(4*(FF//2))
R_W2 = _reg(KF*DH)
R_KS = _reg(SEQ + 8)
R_KV = _reg(2*SEQ)
R_HS = _reg(2*SEQ)
R_B = _reg(NBK*N2*128)
R_Y = _reg(TT*D)
R_O = _reg(TT*DH)
U_ROWS = _off[0]

def kernel(x_hbm, k_hbm, v_hbm, sh_hbm, h_hbm, d_hbm, w1_hbm, w2_hbm, F_hbm, G_hbm, o_hbm,
           U, x_s, k_s, v_s, h_s, w1_s, w2_s, F_s, G_s, sh_s, d_s,
           ht_s, fs_s, o_s, Ax_ref, Ah_ref, ys_ref, ys2_ref, tmp_s, hm_s, sems, zs, *extra):
    copies = {}
    semid = {}
    def mk(name, src, dst):
        if name not in semid: semid[name] = len(semid)
        if _env("NODMA", "0") == "1" and name != "out": return
        c = pltpu.make_async_copy(src, dst, sems.at[semid[name]])
        c.start()
        copies.setdefault(name, []).append(c)
    def wait(name):
        cs = copies.pop(name, [])
        if not cs: return
        if int(_env("SCOPES", "0")):
            with jax.named_scope("wait_" + name):
                for c in cs: c.wait()
        else:
            for c in cs: c.wait()
    def bc(a): return pltpu.bitcast(a, bf16)
    def ub(a): return pltpu.bitcast(a, u32)
    def fb(a): return pltpu.bitcast(a, f32)
    def pk(a, b): return pltpu.pack_elementwise([a, b], packed_dtype=bf16)
    def upk(a, i): return pltpu.unpack_elementwise(a, index=i, packed_dtype=bf16, unpacked_dtype=f32)

    _w = [0] + [int(a) for a in _env('WC', '4,8,11').split(',')] + [14]
    W1C = [(_w[i], _w[i+1]) for i in range(4)]
    def dma_x(name, js):
        for j in js:
            mk(name, x_hbm.at[:, pl.ds(j*128, 128)], x_s.at[pl.ds(j*DH, DH)].bitcast(bf16))
    def dma_w1(name, q):
        for jf in range(*W1C[q]):
            mk(name, w1_hbm.at[:, pl.ds(jf*128, 128)], w1_s.at[pl.ds(jf*DH, DH)].bitcast(bf16))
    def dma_kvh(name, ct):
        lo = ct*128
        n = min(128, D - lo)
        mk(name, k_hbm.at[pl.ds(lo, n)], k_s.at[pl.ds(lo, n)])
        mk(name, v_hbm.at[pl.ds(lo, n)], v_s.at[pl.ds(lo, n)])
        mk(name, h_hbm.at[pl.ds(lo, n)], h_s.at[pl.ds(lo, n)])
    dma_x("g0", [0]); dma_w1("g1", 0)
    dma_x("g2", [1, 2, 3]); dma_w1("g2", 1)
    dma_w1("g3", 2); dma_w1("g3", 3)
    dma_x("g4", range(4, 16))
    mk("g5", sh_hbm, sh_s); mk("g5", d_hbm, d_s)
    mk("g5", F_hbm, F_s); dma_kvh("g5", 0)
    mk("g6", G_hbm, G_s); dma_kvh("g6", 1)
    dma_kvh("g7", 2); dma_kvh("g7", 3)
    for jf in range(KF):
        mk("g7", w2_hbm.at[:, pl.ds(jf*128, 128)], w2_s.at[pl.ds(jf*DH, DH)].bitcast(bf16))

    oL = pl.multiple_of(pl.semaphore_read(zs.at[0]), 8)
    oS = pl.multiple_of(pl.semaphore_read(zs.at[1]), 8)
    oX = pl.multiple_of(pl.semaphore_read(zs.at[2]), 8)
    oY = pl.multiple_of(pl.semaphore_read(zs.at[3]), 8)
    oC = pl.multiple_of(pl.semaphore_read(zs.at[4]), 8)
    Zv = jnp.full((8, 128), oX, jnp.int32).astype(u32)
    LAG = int(_env("LAG", "0"))
    bb = []
    DEP = int(_env("DEP", "1"))
    depq = []; tnow = [0]
    DL = int(_env("DL", "0")); DLT = int(_env("DLT", "600"))
    def bb_in(a):
        acc = None
        while depq and depq[0][0] <= tnow[0]:
            v = depq.pop(0)[1]
            acc = v if acc is None else acc | v
        if acc is None: return a
        for _ in range(int(_env("NROLL", "0"))):
            acc = pltpu.roll(acc, 1, 1)
        return jnp.concatenate([a[:8] | (acc & Zv), a[8:]], axis=0)
    def bb_out(v):
        pass
    def vdep(val, every=1):
        if not DEP: return
        val = val if val.dtype == u32 else ub(val)
        n = val.shape[0]//8
        acc = None
        for i in range(n - 1, -1, -every):
            v = val[8*i:8*i+8]
            acc = v if acc is None else acc | v
        t = tnow[0] + (DL if every == 1 else DLT)
        if depq and depq[-1][0] == t:
            depq[-1] = (t, depq[-1][1] | acc)
        else:
            depq.append((t, acc)); depq.sort(key=lambda x: x[0])
    def Ust(base, val, every=1):
        U[pl.ds(oS + base, val.shape[0]), :] = val if val.dtype == u32 else ub(val)
        if every: vdep(val, every)
    def Uld(base, n, stride=None):
        return U[pl.ds(oS + base, n, stride=stride), :] if stride else U[pl.ds(oS + base, n), :]
    if _env("OS0", "1") == "1": oS = 0
    if _env("PIN", "0") == "0": oL = oS
    if _env("OPQ", "0") == "0": oC = 0
    PINM = _env("PIN", "0")
    def Upin(base, n, stride=None, main=False):
        if PINM == "2":
            if not main: return Uld(base, n, stride)
            st = stride or 1
            a = U[pl.ds(oL + base, 8, stride=stride), :] if stride else U[pl.ds(oL + base, 8), :]
            b = Uld(base + 8*st, n - 8, stride)
            return jnp.concatenate([a, b], axis=0)
        return U[pl.ds(oL + base, n, stride=stride), :] if stride else U[pl.ds(oL + base, n), :]

    if _env("NOZ", "0") == "0":
        U[pl.ds(R_W1T + 3*(FF//2), FF//2), :] = jnp.zeros((FF//2, 128), u32)
        for j in range(TT):
            U[pl.ds(R_XN + j*256 + DH, 32), :] = jnp.zeros((32, 128), u32)
        U[pl.ds(R_KS, 8), :] = jnp.zeros((8, 128), u32)

    def eo_split(t, n):
        tmp_s[pl.ds(0, n), :] = t
        wa = tmp_s[pl.ds(0, n//2, stride=2), :]
        wb = tmp_s[pl.ds(1, n//2, stride=2), :]
        e = pltpu.pack_elementwise([wa, wb], packed_dtype=jnp.uint16)
        o = pltpu.pack_elementwise([wa >> 16, wb >> 16], packed_dtype=jnp.uint16)
        return e, o
    def W1T(jf):
        for kt in range(4):
            w = 128 if kt < 3 else 64
            t = ub(bc(w1_s[pl.ds(jf*DH + kt*64, w//2), :]).T)
            tmp_s[pl.ds(64*kt, 64), pl.ds(0, w)] = t
            wa = tmp_s[pl.ds(64*kt, 32, stride=2), pl.ds(0, w)]
            wb = tmp_s[pl.ds(64*kt + 1, 32, stride=2), pl.ds(0, w)]
            e = pltpu.pack_elementwise([wa, wb], packed_dtype=jnp.uint16)
            o = pltpu.pack_elementwise([wa >> 16, wb >> 16], packed_dtype=jnp.uint16)
            for g in range(4):
                b = R_W1T + kt*(FF//2) + jf*64 + g*16
                U[pl.ds(oS + b, 8), pl.ds(0, w)] = e[g*8:(g+1)*8]
                U[pl.ds(oS + b + 8, 8), pl.ds(0, w)] = o[g*8:(g+1)*8]
    def W2R(kt):
        wa = w2_s[pl.ds(kt*DH, DH//2, stride=2), :]
        wb = w2_s[pl.ds(kt*DH + 1, DH//2, stride=2), :]
        e = pltpu.pack_elementwise([wa, wb], packed_dtype=jnp.uint16)
        o = pltpu.pack_elementwise([wa >> 16, wb >> 16], packed_dtype=jnp.uint16)
        for g in range(D//32):
            Ust(R_W2 + kt*DH + g*16, e[g*8:(g+1)*8])
            Ust(R_W2 + kt*DH + g*16 + 8, o[g*8:(g+1)*8])
    EV_T = int(_env("EVT", "1"))
    lnst = {}
    def LN1(j):
        xu = x_s[pl.ds(j*DH, DH), :]
        xe = upk(xu, 0); xo = upk(xu, 1)
        c = xe[0:1]
        de = xe - c; do = xo - c
        s1 = jnp.sum(de + do, axis=0, keepdims=True)*(1.0/D)
        s2 = jnp.sum(de*de + do*do, axis=0, keepdims=True)*(1.0/D)
        var = jnp.maximum(s2 - s1*s1, 0.0)
        lnst[j] = (c + s1, lax.rsqrt(var + EPS))
    def LN2(j, p, np_):
        m, rs = lnst[j]
        n = DH//np_
        xu = x_s[pl.ds(oX + j*DH + p*n, n), :]
        Ust(R_XN + j*256 + p*n, pk((upk(xu, 0) - m)*rs, (upk(xu, 1) - m)*rs))
    def F1(j, a, b):
        R = (b - a)*128
        if _env("SEPL", "0") == "1":
            lhs = jnp.concatenate([bc(w1_s[pl.ds(kt*768 + a*64 % 700, R//2), :]) for kt in range(4)], axis=1)
        else:
            lhs = jnp.concatenate([bc(Upin(R_W1T + kt*(FF//2) + a*64, R//2)) for kt in range(4)], axis=1)
        if _env("SEPR", "0") == "1":
            rhs = bc(bb_in(x_s[pl.ds((j % 12)*256, 256), :]))
        else:
            rhs = bc(bb_in(Upin(R_XN + j*256, 256, main=True)))
        h = jnp.dot(lhs, rhs, preferred_element_type=f32)
        bb_out(h[-8:])
        hh = h*0.5
        h = hh*jnp.tanh(hh) + hh
        h = h.reshape(R//32, 2, 16, 128)
        ht_s[pl.ds(j*(FF//2) + a*64, R//2), :] = pk(h[:, 0].reshape(R//2, 128), h[:, 1].reshape(R//2, 128))
    def F2dot(j, r0, r1):
        lhs = jnp.concatenate([bc(Upin(R_W2 + kt*DH + r0//2, (r1 - r0)//2, main=(kt == 0))) for kt in range(KF)], axis=1)
        rhs = bc(bb_in(ht_s[pl.ds(oC + j*(FF//2), FF//2), :]))
        f = jnp.dot(lhs, rhs, preferred_element_type=f32)
        bb_out(f[-8:])
        return f
    def FINp(j, r0, r1, f, fusedp=False):
        n = (r1 - r0)//2; p0 = r0//2
        f = f.reshape((r1 - r0)//32, 2, 16, 128)
        fe = f[:, 0].reshape(n, 128); fo = f[:, 1].reshape(n, 128)
        xu = x_s[pl.ds(oY + j*DH + p0, n), :]
        xn = Upin(R_XN + j*256 + p0, n)
        ye = fb(Upin(R_Y + j*D + r0, n, stride=2)); yo = fb(Upin(R_Y + j*D + r0 + 1, n, stride=2))
        oe = upk(xu, 0) + upk(xn, 0)*ye + fe
        oo = upk(xu, 1) + upk(xn, 1)*yo + fo
        if fusedp:
            o_s[pl.ds(j*DH + p0, n), :] = pk(oe, oo)
        else:
            Ust(R_O + j*DH + p0, pk(oe, oo))
    def F2a(j, r0, r1):
        fs_s[pl.ds(j*D + r0, r1 - r0), :] = F2dot(j, r0, r1)
    def FINd(j, r0, r1):
        FINp(j, r0, r1, fs_s[pl.ds(oC + j*D + r0, r1 - r0), :])
    def F2f(j, r0, r1):
        FINp(j, r0, r1, F2dot(j, r0, r1), True)
    def OUT(j, fusedp=False):
        src = o_s.at[pl.ds(j*DH, DH)] if fusedp else U.at[pl.ds(R_O + j*DH, DH)]
        mk("out", src.bitcast(bf16), o_hbm.at[:, pl.ds(j*128, 128)])
    taps = {}
    def TAPS(ct):
        c0 = c0_of(ct)
        t = sh_s[:, pl.ds(c0, 128)].astype(f32)
        taps[ct] = [t[i:i+1] for i in range(4)] + [d_s[:, pl.ds(c0, 128)].astype(f32)]
    def Ak(ct, r):
        c0 = c0_of(ct)
        Ust(R_KS + r*128 + 8, k_s[pl.ds(c0, 128), pl.ds(r*128, 128)].T.astype(f32), EV_T)
    def Akv(ct, r):
        c0 = c0_of(ct)
        t0, t1, t2, t3, _ = taps[ct]
        r0 = R_KS + r*128
        vv = v_s[pl.ds(c0, 128), pl.ds(r*128, 128)].T.astype(f32)
        acc = fb(Uld(r0 + 5, 128))*t3 + fb(Uld(r0 + 6, 128))*t2
        acc = acc + fb(Uld(r0 + 7, 128))*t1
        acc = acc + fb(Uld(r0 + 8, 128))*t0
        Ust(R_KV + (ct % 2)*SEQ + r*128, acc*vv)
    def Ah(ct, r):
        c0 = c0_of(ct)
        Ust(R_HS + (ct % 2)*SEQ + r*128, h_s[pl.ds(c0, 128), pl.ds(r*128, 128)].T.astype(f32), EV_T)
    def C(ct, n2):
        rhs = [fb((bb_in if b == 0 else (lambda a: a))(Upin(R_KV + (ct % 2)*SEQ + b*L + n2, 128, stride=N2, main=(b == 0)))) for b in range(NBK)]
        rhs += [fb(Upin(R_HS + (ct % 2)*SEQ + b*L + n2, 128, stride=N2)) for b in range(NBK)]
        A = jnp.dot(bc(F_s[pl.ds(n2*128, 128), :]), jnp.concatenate(rhs, axis=1).astype(bf16), preferred_element_type=f32)
        bb_out(A[-8:, -128:])
        for b in range(NBK):
            Ax_ref[pl.ds((b*N2 + n2)*256, 256), :] = A[:, b*128:(b+1)*128]
            Ah_ref[pl.ds((b*N2 + n2)*256, 256), :] = A[:, (NBK+b)*128:(NBK+b+1)*128]
    DM = _env("DM", "reg")
    def Dpieces(ct, j):
        r0 = j*8
        st = {}
        hb = (j % 2)*256
        def ld(ref, b):
            return [(ref[pl.ds(oC + (b*N2 + n)*256 + r0, 8), :], ref[pl.ds(oC + (b*N2 + n)*256 + r0 + 128, 8), :]) for n in range(N2)]
        def ph(b):
            h = ld(Ah_ref, b)
            if b == 0:
                h[0] = (h[0][0] + taps[ct][4], h[0][1])
            H = dft4(h, 1)
            if DM == "reg":
                st["H", b] = H
            else:
                for k in range(N2):
                    hm_s[pl.ds(hb + (b*4 + k)*16, 16), :] = jnp.concatenate([H[k][0], H[k][1]], axis=0)
        def px(b):
            st["X", b] = dft4(ld(Ax_ref, b), 1)
        def pm(k2):
            X = [st["X", b] for b in range(NBK)]
            if DM == "reg":
                Hk = [st["H", b][k2] for b in range(NBK)]
            else:
                Hk = [(hm_s[pl.ds(oY + hb + (b*4 + k2)*16, 8), :], hm_s[pl.ds(oY + hb + (b*4 + k2)*16 + 8, 8), :]) for b in range(NBK)]
            Y = []
            for a in range(NBK):
                acc = cmul(X[0][k2], Hk[a])
                for b in range(1, a+1):
                    acc = cadd(acc, cmul(X[b][k2], Hk[a-b]))
                Y.append(acc)
            for a in range(NBK):
                X[a][k2] = Y[a] if a == 0 else (Y[a][0] + Y[a-1][1], Y[a][1] - Y[a-1][0])
            lk = _env("LK", "3")
            if lk == "a":
                for a in range(NBK): vdep(X[a][k2][0]); vdep(X[a][k2][1])
            elif lk == "3":
                vdep(X[3][k2][0]); vdep(X[3][k2][1])
            elif lk == "23":
                for a in (2, 3): vdep(X[a][k2][0]); vdep(X[a][k2][1])
        def pi_(a):
            Bq = dft4(st["X", a], -1)
            for n in range(N2):
                if _env("BSEP", "0") == "1":
                    v_ = pk(Bq[n][0], Bq[n][1])
                    o_s[pl.ds((a*N2 + n)*128 + j*8, 8), :] = v_
                    vdep(v_, 1)
                else:
                    Ust(R_B + (a*N2 + n)*128 + j*8, pk(Bq[n][0], Bq[n][1]))
        out = []
        for b in range(NBK): out.append((lambda b=b: ph(b), 0, 17))
        for b in range(NBK): out.append((lambda b=b: px(b), 0, 16))
        for k2 in range(N2): out.append((lambda k2=k2: pm(k2), 0, 78))
        for a in range(NBK): out.append((lambda a=a: pi_(a), 0, 20))
        return out
    def E(ct, n2):
        g = jnp.concatenate([bc(G_s[pl.ds((n2*2 + kt)*64, 64), :]) for kt in range(2)], axis=1)
        rhs = jnp.concatenate([bc((bb_in if b == 0 else (lambda a: a))(Upin(R_B + (b*N2 + n2)*128, 128, main=(b == 0)))) for b in range(NBK)], axis=1)
        y = jnp.dot(g, rhs, preferred_element_type=f32)
        bb_out(y[-8:, -128:])
        for b in range(NBK):
            (ys_ref, ys2_ref)[ct % 2][pl.ds(b*L + n2, 128, stride=N2), :] = y[:, b*128:(b+1)*128]
    def Fy(ct, r):
        c0 = c0_of(ct)
        yt = (ys_ref, ys2_ref)[ct % 2][pl.ds(oC + r*128, 128), :].T
        if ct < 3:
            Ust(R_Y + r*D + c0, yt, EV_T)
        else:
            Ust(R_Y + r*D + 384, yt[64:], EV_T)

    def It(fn, m=0, v=0): return (fn, m, v)
    def W(name): return It(lambda: wait(name))
    def weave(ms, vs):
        if not ms: return list(vs)
        if not vs: return list(ms)
        M = sum(i[1] for i in ms); Vt = sum(max(i[2], 1) for i in vs)
        out = []; ma = 0.0; va = 0.0; vi = 0
        for it in ms:
            ma += it[1]
            while vi < len(vs) and (va + 0.5*max(vs[vi][2], 1))/Vt <= (ma - 0.5*it[1])/M:
                out.append(vs[vi]); va += max(vs[vi][2], 1); vi += 1
            out.append(it)
        out += vs[vi:]
        return out
    def vmerge(a, b):
        if not a: return list(b)
        if not b: return list(a)
        A = sum(max(x[2], 1) for x in a); B = sum(max(x[2], 1) for x in b)
        out = []; ia = ib = 0; ta = tb = 0.0
        while ia < len(a) or ib < len(b):
            fa = (ta + 0.5*max(a[ia][2], 1))/A if ia < len(a) else 2
            fb_ = (tb + 0.5*max(b[ib][2], 1))/B if ib < len(b) else 2
            if fa <= fb_: out.append(a[ia]); ta += max(a[ia][2], 1); ia += 1
            else: out.append(b[ib]); tb += max(b[ib][2], 1); ib += 1
        return out
    def weave2(ms, vs):
        mm = [x for x in ms if x[1] > 0]
        if not mm or not vs: return ms + vs
        o = weave(mm, vs)
        pre = {}; cur = []
        for x in ms:
            if x[1] > 0:
                pre[id(x)] = cur; cur = []
            else:
                cur.append(x)
        oo = []
        for x in o:
            if id(x) in pre: oo += pre[id(x)]
            oo.append(x)
        return oo + cur
    def spread(a, b):
        if not a: return list(b)
        if not b: return list(a)
        A = sum(x[1] for x in a); B = sum(x[1] for x in b)
        out = []; ia = ib = 0; ta = tb = 0.0
        while ia < len(a) or ib < len(b):
            fa = (ta + 0.5*a[ia][1])/A if ia < len(a) else 2
            fb_ = (tb + 0.5*b[ib][1])/B if ib < len(b) else 2
            if ia < len(a) and a[ia][1] == 0: fa = -1
            if ib < len(b) and b[ib][1] == 0: fb_ = -1
            if fa <= fb_: out.append(a[ia]); ta += a[ia][1]; ia += 1
            else: out.append(b[ib]); tb += b[ib][1]; ib += 1
        return out
    def gA(ct):
        it = [It(lambda: TAPS(ct), 0, 10), It(lambda: Ak(ct, 0), 0, 40)]
        for r in range(TT):
            if r + 1 < TT:
                it.append(It(lambda r=r: Ak(ct, r+1), 0, 40))
            it.append(It(lambda r=r: Akv(ct, r), 0, 170))
            it.append(It(lambda r=r: Ah(ct, r), 0, 40))
        return it
    def gD(ct): return [p for j in range(16) for p in Dpieces(ct, j)]
    def gFy(ct): return [It(lambda r=r: Fy(ct, r), 0, 20) for r in range(16)]
    def gC(ct): return [It(lambda n=n: C(ct, n), 512, 64) for n in range(N2)]
    def gE(ct): return [It(lambda n=n: E(ct, n), 256, 64) for n in range(N2)]
    SUB = int(_env("SUB", "1"))
    R2 = int(_env("R2", "96"))
    NLN = int(_env("NLN", "2"))
    def iF1s(j, a, b):
        return [It(lambda a0=a0: F1(j, a0, min(b, a0 + SUB)), (min(b, a0 + SUB) - a0)*128, 0) for a0 in range(a, b, SUB)]
    def iF1(j, q): return It(lambda: F1(j, *W1C[q]), (W1C[q][1] - W1C[q][0])*128, 0)
    def gLN(j): return [It(lambda: LN1(j), 0, 300)] + [It(lambda p=p: LN2(j, p, NLN), 0, 200//NLN) for p in range(NLN)]
    def iW1T(jf): return It(lambda: W1T(jf), 0, 80)
    def rows2():
        out = []; r = 0
        while r < D:
            n = min(R2, D - r)
            if D - r - n < 32 and D - r - n > 0: n = D - r
            out.append((r, r + n)); r += n
        return out

    FYX = int(_env("FYX", "1"))
    NDEF = int(_env("NDEF", "7"))
    fillers = [it for j in range(4, 16) for it in iF1s(j, 0, KF)]
    fillers += [It(lambda j=j, r0=r0, r1=r1: F2a(j, r0, r1), (r1 - r0)*14//4, 0) for j in range(NDEF) for (r0, r1) in rows2()]
    fpos = [0]
    def take(cyc):
        out = []; acc = 0
        while fpos[0] < len(fillers) and acc < cyc:
            it = fillers[fpos[0]]; fpos[0] += 1
            out.append(it); acc += it[1]
        return out

    P = [int(a) for a in _env("P", "3000,0,1000,5500,500").split(",")]
    P_A0, P_SL, P_X, P_D, P_E3 = P
    segs = []
    s0 = [W("g0")] + gLN(0) + [W("g1")] + [iW1T(jf) for jf in range(*W1C[0])]
    s0 += [iF1(0, 0), W("g2")] + gLN(1)
    s0 += weave([iF1(1, 0), iF1(2, 0), iF1(3, 0)], gLN(2) + gLN(3) + [iW1T(jf) for jf in range(*W1C[1])])
    s0 += [W("g3")]
    s0 += weave2([x for j in range(4) for x in iF1s(j, *W1C[1])], [iW1T(jf) for jf in range(W1C[2][0], W1C[3][1])])
    _m = [x for q in (2, 3) for j in range(4) for x in iF1s(j, *W1C[q])]
    _k = int(_env("G4", "0"))
    s0 += _m[:_k] + [W("g4")]
    s0 += weave2(_m[_k:], [x for j in range(4, 12) for x in gLN(j)])
    s0 += [W("g5")]
    s0 += weave2(take(P_A0), vmerge([x for j in range(12, 16) for x in gLN(j)], gA(0)))
    segs.append(("S", s0))
    for t in range(NT + 1):
        if t >= 1 and t < NT: cm = [x for pair in zip(gE(t-1), gC(t)) for x in pair]
        elif t == 0: cm = gC(0)
        else: cm = gE(t-1)
        pre = []
        if t == 0: pre = [W("g6")]
        if t == 1: pre = [W("g7")]
        vs = gA(t+1) if t + 1 < NT else []
        if t == 1: vs = vmerge(vs, [It(lambda kt=kt: W2R(kt), 0, 70) for kt in range(KF)])
        if t >= 2 and FYX: vs = vmerge(vs, gFy(t-2))
        ms = take(P_SL) + spread(cm, take((P_X if t < 3 else int(_env('PX3', '1000'))) if t < NT else P_E3))
        segs.append((f"X{t}", pre + weave2(ms, vs)))
        if t < NT:
            vs = vmerge(gD(t), gFy(t-1) if (t >= 1 and not FYX) else [])
            segs.append((f"D{t}", weave2(take(P_D), vs)))
    rest = take(10**9)
    fused = []
    for j in range(NDEF, TT):
        fused += [It(lambda j=j, r0=r0, r1=r1: F2f(j, r0, r1), (r1 - r0)*14//4, 0) for (r0, r1) in rows2()] + [It(lambda j=j: OUT(j, True))]
    vs = gFy(NT-1)
    vd = []
    for j in range(NDEF):
        vd += [It(lambda j=j, r0=r0, r1=r1: FINd(j, r0, r1), 0, 100) for (r0, r1) in rows2()] + [It(lambda j=j: OUT(j), 0, 1)]
    segs.append(("Y", weave2(rest, vs)))
    segs.append(("Z", weave2(fused, vd)))
    only = _env("ONLY", "")
    if (only and _env("NOW", "0") == "0") or int(_env("WAITALL", "0")):
        for name in list(copies.keys()):
            wait(name)
    if only:
        if _env("NOTAP", "0") == "0": TAPS(0); TAPS(1); TAPS(2); TAPS(3)
        segs = [sg for sg in segs if sg[0] in only.split(",")]
        print("SEGS", [(n, sum(i[1] for i in it), sum(i[2] for i in it)) for n, it in segs])
    BG = int(_env("BG", "1000000"))
    for si_, (nm, items) in enumerate(segs):
        if si_ > 0 and not (items[0][2] == 0 and items[0][1] == 0 and nm in ("X0", "X1")):
            pl.semaphore_signal(zs.at[5], 1); pl.semaphore_wait(zs.at[5], 1)
        del depq[:]
        acc = 0
        if int(_env("SCOPES", "0")):
            cur = []; parts = []
            for it in items:
                if cur and ((it[1] == 0 and it[2] == 0) or (nm in _env("FINE", "").split(",") and cur[-1][1] > 0)): parts.append(cur); cur = []
                cur.append(it)
            parts.append(cur)
            for pi2, part in enumerate(parts):
                with jax.named_scope(f"s{si_:02d}{nm}_{pi2:02d}"):
                    for it in part:
                        it[0](); tnow[0] += it[1]
            continue
        for ii, it in enumerate(items):
            it[0](); tnow[0] += it[1]; acc += it[1]
            if acc >= BG and nm[0] in _env("BGS", "SXDYZ") and ii + 1 < len(items):
                acc = 0; del depq[:]
                pl.semaphore_signal(zs.at[5], 1); pl.semaphore_wait(zs.at[5], 1)
    if only and _env("SINK", "dma") == "ld":
        o_s[pl.ds(3000, 8), :] = o_s[pl.ds(oY, 8), :] + ht_s[pl.ds(oY, 8), :] + U[pl.ds(oY + R_B, 8), :] + ub(Ax_ref[pl.ds(oY, 8), :]) + ub(Ah_ref[pl.ds(oY, 8), :]) + ub(ys_ref[pl.ds(oY, 8), :]) + ub(fs_s[pl.ds(oY, 8), :])
        OUT(13, True)
    elif only:
        mk("out", U, extra[0]); mk("out", ht_s, extra[1]); mk("out", fs_s, extra[2]); mk("out", Ax_ref, extra[3]); mk("out", Ah_ref, extra[4]); mk("out", ys_ref, extra[5])
    for name in list(copies.keys()):
        wait(name)

@jax.jit
def pallas_parallel_sum__ssm_conv_h3__dense_activation_silu__prompt_kernel(A_q, A_k, A_v, A_shift_k, A_ssm_k, A_ssm_D, B_x, B_w1, B_w2):
    hbm = pl.BlockSpec(memory_space=pltpu.HBM)
    V = pltpu.VMEM
    out = pl.pallas_call(
        kernel,
        out_shape=jax.ShapeDtypeStruct((D, SEQ), bf16),
        in_specs=[hbm]*10,
        out_specs=hbm,
        scratch_shapes=[
            V((U_ROWS, 128), u32),
            V((TT*DH, 128), u32), V((D, SEQ), bf16), V((D, SEQ), bf16), V((D, SEQ), bf16),
            V((KF*DH, 128), u32), V((KF*DH, 128), u32),
            V((N2*128, 128), u32), V((N2*2*64, 128), u32),
            V((4, D), bf16), V((1, D), bf16),
            V((TT*(FF//2), 128), u32), V((TT*D, 128), f32), V((TT*DH, 128), u32),
            V((NBK*N2*256, 128), f32), V((NBK*N2*256, 128), f32),
            V((SEQ + YP, 128), f32), V((SEQ, 128), f32), V((256, 128), u32), V((512, 128), f32),
            pltpu.SemaphoreType.DMA((10,)), pltpu.SemaphoreType.REGULAR((6,)),
        ] + ([V((U_ROWS, 128), u32), V((TT*(FF//2), 128), u32), V((TT*D, 128), f32), V((NBK*N2*256, 128), f32), V((NBK*N2*256, 128), f32), V((2*SEQ, 128), f32)] if _env("ONLY", "") else []),
        compiler_params=pltpu.CompilerParams(vmem_limit_bytes=120*1024*1024, flags=({f: True for f in _env('FLG','').split(',')} if _env('FLG','') else None)),
    )(A_q[0].T, A_k[0].T, A_v[0].T, A_shift_k.T, A_ssm_k, A_ssm_D.reshape(1, D), B_w1, B_w2.T, _F, _G)
    return out.T.reshape(1, SEQ, D)
```
